```python
import os as _os
_os.environ.setdefault("JAX_PLATFORMS", "cpu")
import jax
import jax.numpy as jnp

def _softmax(x, axis=-1):
    return jax.nn.softmax(x, axis=axis)
def _gelu(x):
    return jax.nn.gelu(x, approximate=True)
def _silu(x):
    return jax.nn.silu(x)
def _sigmoid(x):
    return jax.nn.sigmoid(x)
def _layernorm(x, axis=-1, eps=1e-5):
    m = jnp.mean(x, axis=axis, keepdims=True)
    v = jnp.var(x, axis=axis, keepdims=True)
    return (x - m) / jnp.sqrt(v + eps)
def _scatter_add(tgt, idx, src, axis=0):
    return tgt.at[idx].add(src)
def _segment_sum(src, seg, n):
    return jax.ops.segment_sum(src, seg, n)
class _Rng:
    def __init__(self, key):
        self._k = key
    def _next(self):
        self._k, sub = jax.random.split(self._k)
        return sub
    def normal(self, shape):
        return jax.random.normal(self._next(), shape, dtype=jnp.bfloat16)
    def randint(self, lo, hi, shape):
        return jax.random.randint(self._next(), shape, lo, hi, dtype=jnp.int32)
    def uniform(self, shape, lo=0.0, hi=1.0):
        return jax.random.uniform(self._next(), shape, jnp.bfloat16, lo, hi)
    def permutation(self, n):
        return jax.random.permutation(self._next(), n)


kernel_name = 'concat_heads__mha_block_cached__gqa_block_cached__near_ridge'

def setup_inputs():
    _rng = _Rng(jax.random.key(int.from_bytes(__import__("os").urandom(4), "little")))
    _w = (lambda a: (lambda t: t.astype(jnp.bfloat16) if jnp.issubdtype(t.dtype, jnp.floating) else t)(jnp.asarray(a)))
    def _A_setup():
        B, Sq, D = 8, 128, 512
        H, Sk, Dh = 32, 1024, 128
        return {
            "x": _w((lambda *s: _rng.normal(s) * 0.8)(B, Sq, D)),
            "k_cache": _w((lambda *s: _rng.normal(s) * 0.8)(B, H, Sk, Dh)),
            "v_cache": _w((lambda *s: _rng.normal(s) * 0.05)(B, H, Sk, Dh)),
            "wq": _w((lambda *s: _rng.normal(s) * 0.8)(D, H * Dh) * (D ** -0.5)),
            "wo": _w((lambda *s: _rng.normal(s) * 0.05)(H * Dh, D) * ((H * Dh) ** -0.5)),
        }
    _A_in = _A_setup()

    def _B_setup():
        B, Sq, D = 8, 128, 512
        Hq, Hkv, Sk, Dh = 32, 32, 1024, 128
        assert Hq % Hkv == 0, (Hq, Hkv)
        return {
            "x": _w((lambda *s: _rng.normal(s) * 0.8)(B, Sq, D)),
            "k_cache": _w((lambda *s: _rng.normal(s) * 0.8)(B, Hkv, Sk, Dh)),
            "v_cache": _w((lambda *s: _rng.normal(s) * 0.05)(B, Hkv, Sk, Dh)),
            "wq": _w((lambda *s: _rng.normal(s) * 0.8)(D, Hq * Dh) * (D ** -0.5)),
            "wo": _w((lambda *s: _rng.normal(s) * 0.05)(Hq * Dh, D) * ((Hq * Dh) ** -0.5)),
        }
    _B_in = _B_setup()

    return {
        "A_x": _A_in["x"],
        "A_k_cache": _A_in["k_cache"],
        "A_v_cache": _A_in["v_cache"],
        "A_wq": _A_in["wq"],
        "A_wo": _A_in["wo"],
        "B_x": _B_in["x"],
        "B_k_cache": _B_in["k_cache"],
        "B_v_cache": _B_in["v_cache"],
        "B_wq": _B_in["wq"],
        "B_wo": _B_in["wo"],
    }

def reference(A_x, A_k_cache, A_v_cache, A_wq, A_wo, B_x, B_k_cache, B_v_cache, B_wq, B_wo):
    def _A_ref(x, k_cache, v_cache, wq, wo):
        B, Sq, D = x.shape
        H, Dh = 32, 128
        q = (lambda x, *d: x.transpose(*d))((x @ wq).reshape(B, Sq, H, Dh), 0, 2, 1, 3)
        scores = jnp.einsum("bhqd,bhkd->bhqk", q, k_cache) * (Dh ** -0.5)
        p = _softmax(scores, axis=-1)
        o = jnp.einsum("bhqk,bhkd->bhqd", p, v_cache)
        return (lambda x, *d: x.transpose(*d))(o, 0, 2, 1, 3).reshape(B, Sq, H * Dh) @ wo

    def _B_ref(x, k_cache, v_cache, wq, wo):
        B, Sq, D = x.shape
        Hq, Dh = 32, 128
        Hkv = k_cache.shape[1]
        rep = Hq // Hkv
        q = (lambda x, *d: x.transpose(*d))((x @ wq).reshape(B, Sq, Hq, Dh), 0, 2, 1, 3)
        k = jnp.repeat(k_cache, rep, axis=1)
        v = jnp.repeat(v_cache, rep, axis=1)
        scores = jnp.einsum("bhqd,bhkd->bhqk", q, k) * (Dh ** -0.5)
        p = _softmax(scores, axis=-1)
        o = jnp.einsum("bhqk,bhkd->bhqd", p, v)
        return (lambda x, *d: x.transpose(*d))(o, 0, 2, 1, 3).reshape(B, Sq, Hq * Dh) @ wo

    a = _A_ref(A_x, A_k_cache, A_v_cache, A_wq, A_wo)
    b = _B_ref(B_x, B_k_cache, B_v_cache, B_wq, B_wo)
    return jnp.concatenate([a, b], axis=-1)
```

```python
import jax
import jax.numpy as jnp
from jax import lax
import jax.experimental.pallas as pl
import jax.experimental.pallas.tpu as pltpu

LOG2E = 1.4426950408889634
B, SQ, D, H, SK, DH = 8, 128, 512, 32, 1024, 128

def make(G=4, NB=3, P=4, vmem_mb=100):
    NG = H // G
    NS = NG * B
    scale = (DH ** -0.5) * LOG2E

    def kern(ax, ak, av, awq, awo, bx, bk, bv, bwq, bwo, out,
             kv, xb, wqb, wob, acc, ob, kvsem, xsem, wsem, osem):
        xs, ks, vs, wqs, wos = (ax, bx), (ak, bk), (av, bv), (awq, bwq), (awo, bwo)

        def kv_cp(s, br):
            hg = s // B
            b = s % B
            slot = s % NB
            return [pltpu.make_async_copy(src[br].at[b, pl.ds(hg * G + j * P, P)], kv.at[slot, br, i, pl.ds(j * P, P)], kvsem.at[slot, br, j * 2 + i])
                    for j in range(G // P) for i, src in enumerate((ks, vs))]

        def wq_cp(hg, br):
            return pltpu.make_async_copy(wqs[br].at[:, pl.ds(pl.multiple_of(hg * G * DH, G * DH), G * DH)], wqb.at[hg % 2, br], wsem.at[hg % 2, br, 0])

        def wo_cp(hg, br):
            return pltpu.make_async_copy(wos[br].at[pl.ds(pl.multiple_of(hg * G * DH, G * DH), G * DH), :], wob.at[hg % 2, br], wsem.at[hg % 2, br, 1])

        def x_cp(br):
            return pltpu.make_async_copy(xs[br], xb.at[br], xsem.at[br])

        def o_cp(b):
            return pltpu.make_async_copy(ob.at[b], out.at[b], osem.at[b])

        for br in range(2):
            x_cp(br).start()
            wq_cp(0, br).start()
            for c in kv_cp(0, br): c.start()
            wo_cp(0, br).start()
        for s in range(1, NB - 1):
            for br in range(2):
                for c in kv_cp(s, br): c.start()

        def body(s, _):
            hg = s // B
            b = s % B
            slot = s % NB
            ws = hg % 2

            @pl.when(jnp.logical_and(b == 0, hg + 1 < NG))
            def _():
                for br in range(2):
                    wq_cp(hg + 1, br).start()
                    wo_cp(hg + 1, br).start()

            @pl.when(s + NB - 1 < NS)
            def _():
                for br in range(2):
                    for c in kv_cp(s + NB - 1, br): c.start()

            for br in range(2):
                @pl.when(s == 0)
                def _():
                    x_cp(br).wait()

                @pl.when(b == 0)
                def _():
                    wq_cp(hg, br).wait()
                    wo_cp(hg, br).wait()
                cps = kv_cp(s, br)
                q = jnp.dot(xb[br, b], wqb[ws, br], preferred_element_type=jnp.float32)
                q = (q * scale).astype(jnp.bfloat16)
                os = []
                for h in range(G):
                    if h % P == 0:
                        cps[h // P * 2].wait()
                        cps[h // P * 2 + 1].wait()
                    qh = q[:, h * DH:(h + 1) * DH]
                    sc = lax.dot_general(qh, kv[slot, br, 0, h], (((1,), (1,)), ((), ())),
                                         preferred_element_type=jnp.float32)
                    m = jnp.max(sc, axis=-1, keepdims=True)
                    p = jnp.exp2(sc - m)
                    l = jnp.sum(p, axis=-1, keepdims=True)
                    o = jnp.dot(p.astype(jnp.bfloat16), kv[slot, br, 1, h], preferred_element_type=jnp.float32)
                    os.append((o * pl.reciprocal(l, approx=True)).astype(jnp.bfloat16))
                o = jnp.concatenate(os, axis=-1)
                r = jnp.dot(o, wob[ws, br], preferred_element_type=jnp.float32)
                cols = pl.ds(br * D, D)

                @pl.when(hg == 0)
                def _():
                    acc[b, :, cols] = r

                @pl.when(jnp.logical_and(hg > 0, hg < NG - 1))
                def _():
                    acc[b, :, cols] += r

                @pl.when(hg == NG - 1)
                def _():
                    ob[b, :, cols] = (acc[b, :, cols] + r).astype(ob.dtype)

            @pl.when(hg == NG - 1)
            def _():
                o_cp(b).start()

        lax.fori_loop(0, NS, body, None)
        for b in range(B):
            o_cp(b).wait()

    def f(*a):
        return pl.pallas_call(
            kern,
            in_specs=[pl.BlockSpec(memory_space=pl.ANY)] * 10,
            out_specs=pl.BlockSpec(memory_space=pl.ANY),
            out_shape=jax.ShapeDtypeStruct((B, SQ, 2 * D), jnp.bfloat16),
            scratch_shapes=[
                pltpu.VMEM((NB, 2, 2, G, SK, DH), jnp.bfloat16),
                pltpu.VMEM((2, B, SQ, D), jnp.bfloat16),
                pltpu.VMEM((2, 2, D, G * DH), jnp.bfloat16),
                pltpu.VMEM((2, 2, G * DH, D), jnp.bfloat16),
                pltpu.VMEM((B, SQ, 2 * D), jnp.float32),
                pltpu.VMEM((B, SQ, 2 * D), jnp.bfloat16),
                pltpu.SemaphoreType.DMA((NB, 2, 2 * G // P)),
                pltpu.SemaphoreType.DMA((2,)),
                pltpu.SemaphoreType.DMA((2, 2, 2)),
                pltpu.SemaphoreType.DMA((B,)),
            ],
            compiler_params=pltpu.CompilerParams(vmem_limit_bytes=vmem_mb * 1024 * 1024),
        )(*a)
    return f


@jax.jit
def pallas_concat_heads__mha_block_cached__gqa_block_cached__near_ridge_kernel(
    A_x, A_k_cache, A_v_cache, A_wq, A_wo, B_x, B_k_cache, B_v_cache, B_wq, B_wo
):
    return make()(A_x, A_k_cache, A_v_cache, A_wq, A_wo, B_x, B_k_cache, B_v_cache, B_wq, B_wo)
```
